```python
import os as _os
_os.environ.setdefault("JAX_PLATFORMS", "cpu")
import jax
import jax.numpy as jnp

def _softmax(x, axis=-1):
    return jax.nn.softmax(x, axis=axis)
def _gelu(x):
    return jax.nn.gelu(x, approximate=True)
def _silu(x):
    return jax.nn.silu(x)
def _sigmoid(x):
    return jax.nn.sigmoid(x)
def _layernorm(x, axis=-1, eps=1e-5):
    m = jnp.mean(x, axis=axis, keepdims=True)
    v = jnp.var(x, axis=axis, keepdims=True)
    return (x - m) / jnp.sqrt(v + eps)
def _scatter_add(tgt, idx, src, axis=0):
    return tgt.at[idx].add(src)
def _segment_sum(src, seg, n):
    return jax.ops.segment_sum(src, seg, n)
class _Rng:
    def __init__(self, key):
        self._k = key
    def _next(self):
        self._k, sub = jax.random.split(self._k)
        return sub
    def normal(self, shape):
        return jax.random.normal(self._next(), shape, dtype=jnp.bfloat16)
    def randint(self, lo, hi, shape):
        return jax.random.randint(self._next(), shape, lo, hi, dtype=jnp.int32)
    def uniform(self, shape, lo=0.0, hi=1.0):
        return jax.random.uniform(self._next(), shape, jnp.bfloat16, lo, hi)
    def permutation(self, n):
        return jax.random.permutation(self._next(), n)


kernel_name = 'gated_mix__linear_attn_block__mixer_token_mlp__prompt'

def setup_inputs():
    _rng = _Rng(jax.random.key(int.from_bytes(__import__("os").urandom(4), "little")))
    _w = (lambda a: (lambda t: t.astype(jnp.bfloat16) if jnp.issubdtype(t.dtype, jnp.floating) else t)(jnp.asarray(a)))
    def _A_setup():
        B, S, D = 1, 2048, 512
        return {
            "x": _w((lambda *s: _rng.normal(s) * 0.05)(B, S, D)),
            "wqkv": _w((lambda *s: _rng.normal(s) * 0.8)(D, 3 * D)),
            "wo": _w((lambda *s: _rng.normal(s) * 0.05)(D, D)),
        }
    _A_in = _A_setup()

    def _B_setup():
        B, S, D, F = 1, 2048, 512, 1792
        return {
            "x": _w((lambda *s: _rng.normal(s) * 0.05)(B, S, D)),
            "w1": _w((lambda *s: _rng.normal(s) * 0.1)(S, F) * (S ** -0.5)),
            "b1": _w((lambda *s: _rng.normal(s) * 0.1)(F) * 0.02),
            "w2": _w((lambda *s: _rng.normal(s) * 0.1)(F, S) * (F ** -0.5)),
            "b2": _w((lambda *s: _rng.normal(s) * 0.1)(S) * 0.02),
        }
    _B_in = _B_setup()

    return {
        "A_x": _A_in["x"],
        "A_wqkv": _A_in["wqkv"],
        "A_wo": _A_in["wo"],
        "B_x": _B_in["x"],
        "B_w1": _B_in["w1"],
        "B_b1": _B_in["b1"],
        "B_w2": _B_in["w2"],
        "B_b2": _B_in["b2"],
        "gate_w": _w((lambda *s: _rng.normal(s) * 0.05)(512) * 16.0),
    }

def reference(A_x, A_wqkv, A_wo, B_x, B_w1, B_b1, B_w2, B_b2, gate_w):
    def _A_ref(x, wqkv, wo):
        B, S, D = x.shape
        H = 32; Dh = D // H
        qkv = (lambda x, *d: x.transpose(*d))((x @ wqkv).reshape(B, S, 3, H, Dh), 2, 0, 3, 1, 4)
        q, k, v = qkv[0], qkv[1], qkv[2]
        phi = lambda t: jnp.where(t > 0, t + 1, jnp.exp(t)) + 1e-6
        pq, pk = phi(q), phi(k)
        kv = jnp.einsum("bhsd,bhse->bhde", pk, v)
        z = jnp.einsum("bhsd->bhd", pk)
        num = jnp.einsum("bhqd,bhde->bhqe", pq, kv)
        den = jnp.einsum("bhqd,bhd->bhq", pq, z)[..., None] + 1e-6
        o = num / den
        return (lambda x, *d: x.transpose(*d))(o, 0, 2, 1, 3).reshape(B, S, D) @ wo

    def _B_ref(x, w1, b1, w2, b2):
        B, S, D = x.shape
        h = _layernorm(x, axis=-1)
        u = jnp.einsum("bsd,sf->bdf", h, w1) + b1
        u = _gelu(u)
        y = jnp.einsum("bdf,fs->bds", u, w2) + b2
        return (lambda x, *d: x.transpose(*d))(y, 0, 2, 1)

    x = A_x
    g = _sigmoid((x * gate_w).sum(-1, keepdims=True))
    a = _A_ref(x, A_wqkv, A_wo)
    b = _B_ref(x, B_w1, B_b1, B_w2, B_b2)
    return g * a + (1 - g) * b
```

```python
import functools, contextlib
import jax
import jax.numpy as jnp
from jax import lax
from jax.experimental import pallas as pl
from jax.experimental.pallas import tpu as pltpu

S, D, F, H, DH = 2048, 512, 1792, 32, 16
BF = jnp.bfloat16
F32 = jnp.float32
U32 = jnp.uint32
NN = (((1,), (0,)), ((), ()))
NT = (((1,), (1,)), ((), ()))


def _dot(a, b, dims=NN):
    return lax.dot_general(a, b, dims, preferred_element_type=F32)


def _phi(t):
    return jnp.where(t > 0, t + 1.0, jnp.exp(t)) + 1e-6


def _gelu(x):
    c = 0.7978845608028654
    return 0.5 * x * (1.0 + jnp.tanh(c * (x + 0.044715 * (x * x * x))))


def ldb(ref, r0, R, c0, C):
    return pltpu.bitcast(ref[r0 // 2:(r0 + R) // 2, c0:c0 + C], BF)


def stb(ref, r0, c0, val):
    R, C = val.shape
    ref[r0 // 2:(r0 + R) // 2, c0:c0 + C] = pltpu.bitcast(val, U32)


def make(UN=256, FN=128, scopes=False, deplag=2, kqn=1, kqmerge=True, lnfirst=True, semchk=True, skip=(), gpos=0, x0n=1,
         flags=None):
    sc = (lambda n: jax.named_scope(n)) if scopes else (lambda n: contextlib.nullcontext())
    NT_ = S // 128
    NU = F // UN
    NF = S // FN

    def kernel(ax_hbm, wqkv_hbm, wo_hbm, w1_hbm, b1_hbm, w2_hbm, b2_hbm, gw_hbm, o_hbm,
               x_v, wqkv_v, wo_v, w1_v, w2_v, b1_v, b2_v, gw_v,
               wT, wvT, woT, xT, hT, pkT, pqT, uu, mT, g_v, G_v, z_v, sems, *outs):
        def cp(src, dst, i):
            return pltpu.make_async_copy(src, dst, sems.at[i])

        def xcp(t0, n, i):
            return cp(ax_hbm.at[0, pl.ds(t0 * 128, n * 128)], x_v.at[pl.ds(t0 * 128, n * 128)], i)

        def wcp(j, i):
            return cp(wqkv_hbm.at[:, pl.ds(j * D, D)], wqkv_v.at[:, pl.ds(j * D, D)], i)

        c_x0 = xcp(0, x0n, 0)
        c_wk = wcp(1, 1)
        c_x1 = xcp(x0n, 4 - x0n, 2)
        g3 = [wcp(0, 3), cp(gw_hbm, gw_v, 3)]
        c_x2 = xcp(4, 12, 4)
        g5 = [wcp(2, 5), cp(wo_hbm, wo_v, 5), cp(b1_hbm, b1_v, 5), cp(w1_hbm, w1_v, 5)]
        g6 = [cp(b2_hbm, b2_v, 6), cp(w2_hbm, w2_v, 6)]
        c_o = [cp(outs[j], o_hbm.at[0, pl.ds(j * FN, FN)], 7) for j in range(NF)]
        for c in [c_x0, c_wk, c_x1] + g3 + [c_x2] + g5 + g6:
            c.start()

        def wtrans(dst, r0, j):
            for m in range(4):
                stb(dst, r0 + m * 128, 0, wqkv_v[:, j * D + m * 128:j * D + (m + 1) * 128].T)

        def xtrans(t):
            stb(xT, 0, t * 128, x_v[t * 128:(t + 1) * 128, :].T)

        def kpost(t, n, kT):
            stb(pkT, 0, t * 128, _phi(kT).astype(BF))

        def qpost(t, n, qT):
            stb(pqT, 0, t * 128, _phi(qT[0:D]).astype(BF))
            g_v[:, t * 128:(t + n) * 128] = jax.nn.sigmoid(qT[D:D + 8])

        def kproj(t, n=1):
            kpost(t, n, _dot(ldb(wT, 0, D, 0, D), ldb(xT, 0, D, t * 128, 128 * n)))

        def qproj(t, n=1):
            qpost(t, n, _dot(ldb(wT, D, D + 16, 0, D), ldb(xT, 0, D, t * 128, 128 * n)))

        def kqproj(t, n=1):
            r = _dot(ldb(wT, 0, 2 * D + 16, 0, D), ldb(xT, 0, D, t * 128, 128 * n))
            kpost(t, n, r[0:D])
            qpost(t, n, r[D:2 * D + 16])

        def ln(t):
            b = ldb(xT, 0, D, t * 128, 128).astype(F32)
            m = jnp.mean(b, axis=0, keepdims=True)
            dl = b - m
            var = jnp.mean(dl * dl, axis=0, keepdims=True)
            stb(hT, 0, t * 128, (dl * lax.rsqrt(var + 1e-5)).astype(BF))

        def gacc(c):
            Gc = _dot(ldb(pkT, 0, D, c * 512, 512), x_v[c * 512:(c + 1) * 512, :])
            if c == 0:
                G_v[...] = Gc
            else:
                G_v[...] += Gc

        with sc("p1a"):
            c_x0.wait()
            for t in range(x0n):
                xtrans(t)
            c_wk.wait()
            wtrans(wT, 0, 1)
            for t in range(x0n):
                kproj(t)
                if lnfirst:
                    ln(t)
        with sc("p1b"):
            c_x1.wait()
            for t in range(x0n, 4):
                xtrans(t)
            for t in range(x0n, 4):
                if lnfirst:
                    ln(t)
                kproj(t)
        with sc("p1c"):
            for c in g3:
                c.wait()
            wtrans(wT, D, 0)
            stb(wT, 2 * D, 0, jnp.broadcast_to(gw_v[...].astype(F32).reshape(1, D), (16, D)).astype(BF))
            for t in range(4):
                qproj(t)
                if not lnfirst:
                    ln(t)
        with sc("p1d"):
            c_x2.wait()
            for c in range(1, 4):
                for t in range(4 * c, 4 * c + 4):
                    xtrans(t)
                if gpos == 0:
                    gacc(c - 1)
                if kqmerge:
                    for t in range(4 * c, 4 * c + 4, kqn):
                        kqproj(t, kqn)
                        for tt in range(t, t + kqn):
                            ln(tt)
                        if gpos == 1 and t == 4 * c:
                            gacc(c - 1)
                else:
                    for t in range(4 * c, 4 * c + 4, kqn):
                        kproj(t, kqn)
                    if gpos == 1:
                        gacc(c - 1)
                    for t in range(4 * c, 4 * c + 4, kqn):
                        qproj(t, kqn)
                        for tt in range(t, t + kqn):
                            ln(tt)

        def uproj(j):
            acc = _dot(ldb(hT, 0, D, 0, S), w1_v[:, j * UN:(j + 1) * UN])
            acc = acc + b1_v[pl.ds(j * UN, UN)].astype(F32).reshape(1, UN)
            stb(uu, 0, j * UN, _gelu(acc).astype(BF))

        def zsum():
            acc = ldb(pkT, 0, D, 0, 128).astype(F32)
            for t in range(1, NT_):
                acc = acc + ldb(pkT, 0, D, t * 128, 128).astype(F32)
            z = jnp.sum(acc, axis=1, keepdims=True)
            z_v[...] = jnp.broadcast_to(z, (D, 128))

        def kvm():
            ri = lax.broadcasted_iota(jnp.int32, (128, 128), 0) // DH
            ci = lax.broadcasted_iota(jnp.int32, (128, 128), 1) // DH
            kvs = []
            for gp in range(4):
                kvT = _dot(ldb(wvT, gp * 128, 128, 0, D), G_v[gp * 128:(gp + 1) * 128, :].astype(BF), NT)
                kvs.append(jnp.where(ri == ci, kvT, 0.0).astype(BF))
            return kvs

        def mmat(kvs):
            for gp in range(4):
                stb(mT, 0, gp * 128, _dot(ldb(woT, 0, D, gp * 128, 128), kvs[gp]).astype(BF))

        def dep_on(ref):
            b = pltpu.bitcast(ref[...], jnp.int32)
            acc = None
            for r in range(b.shape[0] // 8):
                for c in range(b.shape[1] // 128):
                    v = b[r * 8:(r + 1) * 8, c * 128:(c + 1) * 128]
                    acc = v if acc is None else (acc | v)
            return jnp.minimum(acc[0:1, :], 0)

        def pqn(t, dep=None):
            pq = ldb(pqT, 0, D, t * 128, 128).astype(F32)
            tt = (pq * z_v[...]).reshape(H, DH, 128)
            den = jnp.sum(tt, axis=1, keepdims=True) + 1e-6
            r = pl.reciprocal(den, approx=True)
            r = r * (2.0 - den * r)
            grow = g_v[0:1, t * 128:(t + 1) * 128]
            if dep is not None:
                grow = jnp.where(dep > 0, 0.0, grow)
            inv = grow.reshape(1, 1, 128) * r
            stb(pqT, 0, t * 128, (pq.reshape(H, DH, 128) * inv).reshape(D, 128).astype(BF))

        with sc("u"):
            for c in g5:
                c.wait()
            wtrans(wvT, 0, 2)
            for m in range(4):
                stb(woT, m * 128, 0, wo_v[:, m * 128:(m + 1) * 128].T)
            gacc(3)
            zsum()
            uproj(0)
            kvs = kvm()
            uproj(1)
            mmat(kvs)
            for j in range(2, NU):
                uproj(j)

        def fin_mm(j):
            sl = slice(j * FN, (j + 1) * FN)
            y = _dot(ldb(uu, 0, D, 0, F), w2_v[:, sl])
            a = _dot(ldb(mT, 0, D, 0, D), ldb(pqT, 0, D, j * FN, FN))
            return y, a

        def fin_out(j, y, a):
            sl = slice(j * FN, (j + 1) * FN)
            y = y + b2_v[pl.ds(j * FN, FN)].astype(F32).reshape(1, FN)
            omg = 1.0 - g_v[:, sl]
            oT = a + (y.reshape(D // 8, 8, FN) * omg[None]).reshape(D, FN)
            outs[j][...] = oT.astype(BF).T
            c_o[j].start()

        with sc("fin"):
            for c in g6:
                c.wait()
            prev = None
            for j in range(NF):
                for t in range(j * FN // 128, (j + 1) * FN // 128):
                    dep = None
                    if deplag and j >= deplag and t == j * FN // 128:
                        dep = dep_on(outs[j - deplag])
                    pqn(t, dep)
                cur = fin_mm(j)
                if prev is not None:
                    fin_out(j - 1, *prev)
                prev = cur
            fin_out(NF - 1, *prev)
        with sc("tail"):
            for j in range(NF):
                c_o[j].wait()

    @jax.jit
    def fn(A_x, A_wqkv, A_wo, B_x, B_w1, B_b1, B_w2, B_b2, gate_w):
        any_spec = pl.BlockSpec(memory_space=pl.ANY)
        return pl.pallas_call(
            kernel,
            out_shape=jax.ShapeDtypeStruct((1, S, D), BF),
            in_specs=[any_spec] * 8,
            out_specs=any_spec,
            scratch_shapes=[
                pltpu.VMEM((S, D), BF),
                pltpu.VMEM((D, 3 * D), BF),
                pltpu.VMEM((D, D), BF),
                pltpu.VMEM((S, F), BF),
                pltpu.VMEM((F, S), BF),
                pltpu.VMEM((F,), BF),
                pltpu.VMEM((S,), BF),
                pltpu.VMEM((D,), BF),
                pltpu.VMEM((D + 8, D), U32),
                pltpu.VMEM((D // 2, D), U32),
                pltpu.VMEM((D // 2, D), U32),
                pltpu.VMEM((D // 2, S), U32),
                pltpu.VMEM((D // 2, S), U32),
                pltpu.VMEM((D // 2, S), U32),
                pltpu.VMEM((D // 2, S), U32),
                pltpu.VMEM((D // 2, F), U32),
                pltpu.VMEM((D // 2, D), U32),
                pltpu.VMEM((8, S), F32),
                pltpu.VMEM((D, D), F32),
                pltpu.VMEM((D, 128), F32),
                pltpu.SemaphoreType.DMA((8,)),
            ] + [pltpu.VMEM((FN, D), BF)] * NF,
            compiler_params=pltpu.CompilerParams(vmem_limit_bytes=100 * 1024 * 1024,
                                                 disable_semaphore_checks=not semchk, flags=flags),
        )(A_x, A_wqkv, A_wo, B_w1, B_b1, B_w2, B_b2, gate_w)

    return fn


_fn = make()


def pallas_gated_mix__linear_attn_block__mixer_token_mlp__prompt_kernel(A_x, A_wqkv, A_wo, B_x, B_w1, B_b1, B_w2, B_b2, gate_w):
    return _fn(A_x, A_wqkv, A_wo, B_x, B_w1, B_b1, B_w2, B_b2, gate_w)
```

```python
import jax
import jax.numpy as jnp
from jax import lax
from jax.experimental import pallas as pl
from jax.experimental.pallas import tpu as pltpu

S, D, F, H, DH = 2048, 512, 1792, 32, 16
T = 128
NTILE = S // T
CH = 512
UN = 256
BF, F32, U32, I32 = jnp.bfloat16, jnp.float32, jnp.uint32, jnp.int32
NN = (((1,), (0,)), ((), ()))
NT = (((1,), (1,)), ((), ()))


def _dot(a, b, dims=NN):
    return lax.dot_general(a, b, dims, preferred_element_type=F32)


def _phi(t):
    return jnp.where(t > 0, t + 1.0, jnp.exp(t)) + 1e-6


def _gelu(x):
    return 0.5 * x * (1.0 + jnp.tanh(0.7978845608028654 * (x + 0.044715 * (x * x * x))))


def _ldb(ref, r0, rows, c0, cols):
    return pltpu.bitcast(ref[r0 // 2:(r0 + rows) // 2, c0:c0 + cols], BF)


def _stb(ref, r0, c0, val):
    rows, cols = val.shape
    ref[r0 // 2:(r0 + rows) // 2, c0:c0 + cols] = pltpu.bitcast(val, U32)


def _kernel(ax_hbm, wqkv_hbm, wo_hbm, w1_hbm, b1_hbm, w2_hbm, b2_hbm, gw_hbm, o_hbm,
            x_v, wqkv_v, wo_v, w1_v, w2_v, b1_v, b2_v, gw_v,
            wT, wvT, woT, xT, hT, pkT, pqT, uu, mT, g_v, G_v, z_v, sems, *outs):
    def cp(src, dst, i):
        return pltpu.make_async_copy(src, dst, sems.at[i])

    def x_cp(t0, n, i):
        return cp(ax_hbm.at[0, pl.ds(t0 * T, n * T)], x_v.at[pl.ds(t0 * T, n * T)], i)

    def w_cp(j, i):
        return cp(wqkv_hbm.at[:, pl.ds(j * D, D)], wqkv_v.at[:, pl.ds(j * D, D)], i)

    c_x0, c_wk, c_x1 = x_cp(0, 1, 0), w_cp(1, 1), x_cp(1, 3, 2)
    c_q = [w_cp(0, 3), cp(gw_hbm, gw_v, 3)]
    c_x2 = x_cp(4, 12, 4)
    c_u = [w_cp(2, 5), cp(wo_hbm, wo_v, 5), cp(b1_hbm, b1_v, 5), cp(w1_hbm, w1_v, 5)]
    c_y = [cp(b2_hbm, b2_v, 6), cp(w2_hbm, w2_v, 6)]
    c_o = [cp(outs[j], o_hbm.at[0, pl.ds(j * T, T)], 7) for j in range(NTILE)]
    for c in [c_x0, c_wk, c_x1] + c_q + [c_x2] + c_u + c_y:
        c.start()

    def w_transpose(dst, r0, j):
        for m in range(D // 128):
            _stb(dst, r0 + m * 128, 0, wqkv_v[:, j * D + m * 128:j * D + (m + 1) * 128].T)

    def x_tile(t):
        return x_v[t * T:(t + 1) * T, :]

    def x_transpose(t):
        _stb(xT, 0, t * T, x_tile(t).T)

    def proj(t, r0, rows, direct):
        w = _ldb(wT, r0, rows, 0, D)
        if direct:
            return _dot(w, x_tile(t), NT)
        return _dot(w, _ldb(xT, 0, D, t * T, T))

    def k_post(t, kT):
        _stb(pkT, 0, t * T, _phi(kT).astype(BF))

    def q_post(t, qT):
        _stb(pqT, 0, t * T, _phi(qT[0:D]).astype(BF))
        g_v[:, t * T:(t + 1) * T] = jax.nn.sigmoid(qT[D:D + 8])

    def k_proj(t):
        k_post(t, proj(t, 0, D, True))

    def q_proj(t):
        q_post(t, proj(t, D, D + 16, False))

    def kq_proj(t, direct=False):
        r = proj(t, 0, 2 * D + 16, direct)
        k_post(t, r[0:D])
        q_post(t, r[D:2 * D + 16])

    def layer_norm(t):
        b = _ldb(xT, 0, D, t * T, T).astype(F32)
        d = b - jnp.mean(b, axis=0, keepdims=True)
        var = jnp.mean(d * d, axis=0, keepdims=True)
        _stb(hT, 0, t * T, (d * lax.rsqrt(var + 1e-5)).astype(BF))

    def g_acc(c, n0=0, n1=D):
        Gc = _dot(_ldb(pkT, 0, D, c * CH, CH), x_v[c * CH:(c + 1) * CH, n0:n1])
        if c == 0:
            G_v[:, n0:n1] = Gc
        else:
            G_v[:, n0:n1] += Gc

    def never(bits):
        return jnp.minimum(bits[0:1, :], 0)

    def z_sum():
        acc = _ldb(pkT, 0, D, 0, T).astype(F32)
        for t in range(1, NTILE):
            acc = acc + _ldb(pkT, 0, D, t * T, T).astype(F32)
        zb = jnp.broadcast_to(jnp.sum(acc, axis=1, keepdims=True), (D, T))
        z_v[...] = zb
        zi = pltpu.bitcast(zb, I32)
        a = zi[0:8]
        for r in range(1, D // 8):
            a = a | zi[r * 8:(r + 1) * 8]
        return never(a)

    def u_proj(j, after=None):
        acc = _dot(_ldb(hT, 0, D, 0, S), w1_v[:, j * UN:(j + 1) * UN])
        bias = b1_v[pl.ds(j * UN, UN)].astype(F32).reshape(1, UN)
        if after is not None:
            bias = jnp.where(jnp.concatenate([after] * (UN // T), axis=1) > 0, 0.0, bias)
        _stb(uu, 0, j * UN, _gelu(acc + bias).astype(BF))

    def kv_blocks():
        ri = lax.broadcasted_iota(I32, (128, 128), 0) // DH
        ci = lax.broadcasted_iota(I32, (128, 128), 1) // DH
        out = []
        for gp in range(D // 128):
            kvT = _dot(_ldb(wvT, gp * 128, 128, 0, D), G_v[gp * 128:(gp + 1) * 128, :].astype(BF), NT)
            out.append(jnp.where(ri == ci, kvT, 0.0).astype(BF))
        return out

    def m_matrix(kvs):
        for gp in range(D // 128):
            _stb(mT, 0, gp * 128, _dot(_ldb(woT, 0, D, gp * 128, 128), kvs[gp]).astype(BF))

    def out_done(ref):
        b = pltpu.bitcast(ref[...], I32)
        acc = None
        for r in range(b.shape[0] // 8):
            for c in range(b.shape[1] // 128):
                v = b[r * 8:(r + 1) * 8, c * 128:(c + 1) * 128]
                acc = v if acc is None else acc | v
        return never(acc)

    def pq_norm(t, after=None):
        pq = _ldb(pqT, 0, D, t * T, T).astype(F32)
        den = jnp.sum((pq * z_v[...]).reshape(H, DH, T), axis=1, keepdims=True) + 1e-6
        r = pl.reciprocal(den, approx=True)
        r = r * (2.0 - den * r)
        grow = g_v[0:1, t * T:(t + 1) * T]
        if after is not None:
            grow = jnp.where(after > 0, 0.0, grow)
        inv = grow.reshape(1, 1, T) * r
        _stb(pqT, 0, t * T, (pq.reshape(H, DH, T) * inv).reshape(D, T).astype(BF))

    def out_tile(t):
        sl = slice(t * T, (t + 1) * T)
        y = _dot(_ldb(uu, 0, D, 0, F), w2_v[:, sl])
        a = _dot(_ldb(mT, 0, D, 0, D), _ldb(pqT, 0, D, t * T, T))
        y = y + b2_v[pl.ds(t * T, T)].astype(F32).reshape(1, T)
        omg = 1.0 - g_v[:, sl]
        oT = a + (y.reshape(D // 8, 8, T) * omg[None]).reshape(D, T)
        outs[t][...] = oT.astype(BF).T
        c_o[t].start()

    c_x0.wait()
    x_transpose(0)
    c_wk.wait()
    w_transpose(wT, 0, 1)
    k_proj(0)

    c_x1.wait()
    for t in range(1, 4):
        x_transpose(t)
    for t in range(1, 4):
        k_proj(t)

    for c in c_q:
        c.wait()
    g_acc(0, 0, 384)
    w_transpose(wT, D, 0)
    _stb(wT, 2 * D, 0, jnp.broadcast_to(gw_v[...].astype(F32).reshape(1, D), (16, D)).astype(BF))
    for t in range(4):
        layer_norm(t)
        q_proj(t)

    c_x2.wait()
    g_acc(0, 384, D)
    for c in range(1, 4):
        for t in range(4 * c, 4 * c + 4):
            x_transpose(t)
        for t in range(4 * c, 4 * c + 4):
            layer_norm(t)
            kq_proj(t, direct=(t == 4))
        if c < 3:
            g_acc(c)

    for c in c_u:
        c.wait()
    w_transpose(wvT, 0, 2)
    for m in range(D // 128):
        _stb(woT, m * 128, 0, wo_v[:, m * 128:(m + 1) * 128].T)
    g_acc(3)
    z_done = z_sum()
    u_proj(0)
    kvs = kv_blocks()
    u_proj(1)
    m_matrix(kvs)
    for j in range(2, F // UN):
        if j == F // UN - 1:
            for c in c_y:
                c.wait()
        u_proj(j, z_done if j == 2 else None)

    for t in range(NTILE):
        pq_norm(t, out_done(outs[t - 1]) if t > 0 else None)
        out_tile(t)
    for c in c_o:
        c.wait()


def make():
    @jax.jit
    def fn(A_x, A_wqkv, A_wo, B_x, B_w1, B_b1, B_w2, B_b2, gate_w):
        del B_x
        any_spec = pl.BlockSpec(memory_space=pl.ANY)
        return pl.pallas_call(
            _kernel,
            out_shape=jax.ShapeDtypeStruct((1, S, D), BF),
            in_specs=[any_spec] * 8,
            out_specs=any_spec,
            scratch_shapes=[
                pltpu.VMEM((S, D), BF),
                pltpu.VMEM((D, 3 * D), BF),
                pltpu.VMEM((D, D), BF),
                pltpu.VMEM((S, F), BF),
                pltpu.VMEM((F, S), BF),
                pltpu.VMEM((F,), BF),
                pltpu.VMEM((S,), BF),
                pltpu.VMEM((D,), BF),
                pltpu.VMEM((D + 8, D), U32),
                pltpu.VMEM((D // 2, D), U32),
                pltpu.VMEM((D // 2, D), U32),
                pltpu.VMEM((D // 2, S), U32),
                pltpu.VMEM((D // 2, S), U32),
                pltpu.VMEM((D // 2, S), U32),
                pltpu.VMEM((D // 2, S), U32),
                pltpu.VMEM((D // 2, F), U32),
                pltpu.VMEM((D // 2, D), U32),
                pltpu.VMEM((8, S), F32),
                pltpu.VMEM((D, D), F32),
                pltpu.VMEM((D, T), F32),
                pltpu.SemaphoreType.DMA((8,)),
            ] + [pltpu.VMEM((T, D), BF)] * NTILE,
            compiler_params=pltpu.CompilerParams(vmem_limit_bytes=100 * 1024 * 1024),
        )(A_x, A_wqkv, A_wo, B_w1, B_b1, B_w2, B_b2, gate_w)

    return fn


_fn = make()


def pallas_gated_mix__linear_attn_block__mixer_token_mlp__prompt_kernel(A_x, A_wqkv, A_wo, B_x, B_w1, B_b1, B_w2, B_b2, gate_w):
    return _fn(A_x, A_wqkv, A_wo, B_x, B_w1, B_b1, B_w2, B_b2, gate_w)
```

```python
import jax
import jax.numpy as jnp
from jax import lax
from jax.experimental import pallas as pl
from jax.experimental.pallas import tpu as pltpu

S, D, F, H, DH = 2048, 512, 1792, 32, 16
T = 128
NTILE = S // T
CH = 512
UN = 256
BF, F32, U32, I32 = jnp.bfloat16, jnp.float32, jnp.uint32, jnp.int32
NN = (((1,), (0,)), ((), ()))
NT = (((1,), (1,)), ((), ()))


def _dot(a, b, dims=NN):
    return lax.dot_general(a, b, dims, preferred_element_type=F32)


def _phi(t):
    return jnp.where(t > 0, t + 1.0, jnp.exp(t)) + 1e-6


def _gelu(x):
    return 0.5 * x * (1.0 + jnp.tanh(0.7978845608028654 * (x + 0.044715 * (x * x * x))))


def _ldb(ref, r0, rows, c0, cols):
    return pltpu.bitcast(ref[r0 // 2:(r0 + rows) // 2, c0:c0 + cols], BF)


def _stb(ref, r0, c0, val):
    rows, cols = val.shape
    ref[r0 // 2:(r0 + rows) // 2, c0:c0 + cols] = pltpu.bitcast(val, U32)


def _kernel(ax_hbm, wqkv_hbm, wo_hbm, w1_hbm, b1_hbm, w2_hbm, b2_hbm, gw_hbm, o_hbm,
            x_v, wqkv_v, wo_v, w1_v, w2_v, b1_v, b2_v, gw_v,
            wT, wvT, woT, xT, hT, pkT, pqT, uu, mT, g_v, G_v, z_v, gwc_v, sems, *rest):
    ANC, outs = rest[:5], rest[5:]
    def cp(src, dst, i):
        return pltpu.make_async_copy(src, dst, sems.at[i])

    def x_cp(t0, n, i):
        return cp(ax_hbm.at[0, pl.ds(t0 * T, n * T)], x_v.at[pl.ds(t0 * T, n * T)], i)

    def w_cp(j, i):
        return cp(wqkv_hbm.at[:, pl.ds(j * D, D)], wqkv_v.at[:, pl.ds(j * D, D)], i)

    def a_cp(k, i):
        return cp(wo_hbm.at[pl.ds(0, 16), pl.ds(0, T)], ANC[k].at[pl.ds(0, 16)], i)

    grp = {}
    nsem = [0]

    def group(name, *mk):
        if name not in ORDER.split(","):
            return
        i = nsem[0]
        nsem[0] += 1
        grp[name] = [m(i) for m in mk]

    group("x0", lambda i: x_cp(0, 1, i))
    group("wk", lambda i: w_cp(1, i))
    for m in range(4):
        group(f"k{m}", lambda i, m=m: cp(wqkv_hbm.at[:, pl.ds(D + m * 128, 128)], wqkv_v.at[:, pl.ds(D + m * 128, 128)], i))
    group("x03", lambda i: x_cp(0, 4, i))
    group("x01", lambda i: x_cp(0, 2, i))
    group("x23", lambda i: x_cp(2, 2, i))
    for name, t0, n in XS:
        group(name, lambda i, t0=t0, n=n: x_cp(t0, n, i))
    group("q", lambda i: w_cp(0, i), lambda i: cp(gw_hbm, gw_v, i), lambda i: a_cp(1, i))
    group("u", lambda i: w_cp(2, i), lambda i: cp(wo_hbm, wo_v, i), lambda i: cp(b1_hbm, b1_v, i),
          lambda i: cp(w1_hbm, w1_v, i), lambda i: a_cp(3, i))

    def w1_cp(j0, j1, i):
        return cp(w1_hbm.at[:, pl.ds(j0 * UN, (j1 - j0) * UN)], w1_v.at[:, pl.ds(j0 * UN, (j1 - j0) * UN)], i)

    group("us", lambda i: w_cp(2, i), lambda i: cp(wo_hbm, wo_v, i), lambda i: cp(b1_hbm, b1_v, i),
          lambda i: w1_cp(0, W1S[1], i), lambda i: a_cp(3, i))
    for a_, b_ in zip(W1S[1:-1], W1S[2:]):
        group(f"w1_{a_}", lambda i, a_=a_, b_=b_: w1_cp(a_, b_, i))
    group("y", lambda i: cp(b2_hbm, b2_v, i), lambda i: cp(w2_hbm, w2_v, i), lambda i: a_cp(4, i))
    i_out = nsem[0]
    c_o = [cp(outs[j], o_hbm.at[0, pl.ds(j * T, T)], i_out) for j in range(NTILE)]
    for name in ORDER.split(","):
        if name not in LATE:
            for c in grp[name]:
                c.start()

    def wait(name):
        for c in grp.pop(name):
            c.wait()
        for g2, after in LATE.items():
            if after == name:
                for c in grp[g2]:
                    c.start()

    def w_transpose(dst, r0, j):
        for m in range(D // 128):
            _stb(dst, r0 + m * 128, 0, wqkv_v[0:D, j * D + m * 128:j * D + (m + 1) * 128].T)

    def x_tile(t):
        return x_v[t * T:(t + 1) * T, :]

    def x_transpose(t):
        _stb(xT, 0, t * T, x_tile(t).T)

    def proj(t, r0, rows, direct):
        w = _ldb(wT, r0, rows, 0, D)
        rhs = x_tile(t) if direct else _ldb(xT, 0, D, t * T, T)
        if DELAY[0] == ("b", t):
            rhs = gate_on(rhs, delay(g_v[:, 0:T], DELAY[1]))
        if LDEP and (t - LDEP) in ldone:
            rhs = gate_on(rhs, ldone.pop(t - LDEP))
        if direct:
            return _dot(w, rhs, NT)
        return _dot(w, rhs)

    def k_post(t, kT):
        v = _phi(kT).astype(BF)
        _stb(pkT, 0, t * T, v)
        return v

    def q_post(t, qT):
        v = _phi(qT[0:D]).astype(BF)
        _stb(pqT, 0, t * T, v)
        if not VGATE:
            g_v[:, t * T:(t + 1) * T] = jax.nn.sigmoid(qT[D:D + 8])
        return v

    def k_proj(t):
        return k_post(t, proj(t, 0, D, True))

    def q_proj(t):
        return q_post(t, proj(t, D, D + EX, False))

    def kq_proj(t, direct=False):
        r = proj(t, 0, 2 * D + EX, direct)
        k_post(t, r[0:D])
        return q_post(t, r[D:2 * D + EX])

    ldone = {}

    def gate_on(val, after):
        vi = pltpu.bitcast(val, I32)
        reps = vi.shape[1] // T
        m = jnp.concatenate([after] * reps, axis=1) if reps > 1 else after
        return pltpu.bitcast(jnp.where(m > 0, 0, vi), val.dtype)

    def delay(seed, n):
        x = seed
        for _ in range(n):
            x = x * 1.0000001 + 1e-9
        return jnp.minimum(pltpu.bitcast(jnp.abs(x), I32)[0:1, :], 0)

    def layer_norm(t):
        b = _ldb(xT, 0, D, t * T, T).astype(F32)
        d = b - jnp.mean(b, axis=0, keepdims=True)
        var = jnp.mean(d * d, axis=0, keepdims=True)
        hb = pltpu.bitcast((d * lax.rsqrt(var + 1e-5)).astype(BF), I32)
        hT[:, t * T:(t + 1) * T] = pltpu.bitcast(hb, U32)
        if LDEP:
            a = hb[0:8]
            for r in range(1, D // 16):
                a = a | hb[r * 8:(r + 1) * 8]
            ldone[t] = jnp.minimum(a[0:1, :], 0)
        if VGATE:
            lg = jnp.sum(b * gwc_v[...], axis=0, keepdims=True)
            g_v[:, t * T:(t + 1) * T] = jnp.broadcast_to(jax.nn.sigmoid(lg), (8, T))

    def g_acc(c, n0=0, n1=D):
        Gc = _dot(_ldb(pkT, 0, D, c * CH, CH), x_v[c * CH:(c + 1) * CH, n0:n1])
        if c == 0:
            G_v[:, n0:n1] = Gc
        else:
            G_v[:, n0:n1] += Gc

    def never(bits):
        return jnp.minimum(bits[0:1, :], 0)

    def z_sum():
        dep = None
        for rb in range(0, D, ZR):
            acc = _ldb(pkT, rb, ZR, 0, T).astype(F32)
            for t in range(1, NTILE):
                acc = acc + _ldb(pkT, rb, ZR, t * T, T).astype(F32)
            zb = jnp.broadcast_to(jnp.sum(acc, axis=1, keepdims=True), (ZR, T))
            z_v[rb:rb + ZR, :] = zb
            zi = pltpu.bitcast(zb, I32)
            for r in range(ZR // 8):
                dep = zi[r * 8:(r + 1) * 8] if dep is None else dep | zi[r * 8:(r + 1) * 8]
        return never(dep)

    def u_proj(j, after=None):
        if DELAY[0] == ("u", j):
            after = delay(g_v[:, 0:T], DELAY[1])
        if f"w1_{j}" in grp:
            wait(f"w1_{j}")
        acc = _dot(_ldb(hT, 0, D, 0, S), w1_v[0:S, j * UN:(j + 1) * UN])
        bias = b1_v[pl.ds(j * UN, UN)].astype(F32).reshape(1, UN)
        if after is not None:
            bias = jnp.where(jnp.concatenate([after] * (UN // T), axis=1) > 0, 0.0, bias)
        v = _gelu(acc + bias).astype(BF)
        _stb(uu, 0, j * UN, v)
        return v[:, 0:T]

    def kv_blocks():
        ri = lax.broadcasted_iota(I32, (128, 128), 0) // DH
        ci = lax.broadcasted_iota(I32, (128, 128), 1) // DH
        out = []
        for gp in range(D // 128):
            kvT = _dot(_ldb(wvT, gp * 128, 128, 0, D), G_v[gp * 128:(gp + 1) * 128, :].astype(BF), NT)
            out.append(jnp.where(ri == ci, kvT, 0.0).astype(BF))
        return out

    def m_matrix(kvs):
        for gp in range(D // 128):
            _stb(mT, 0, gp * 128, _dot(_ldb(woT, 0, D, gp * 128, 128), kvs[gp]).astype(BF))

    def out_done(ref):
        b = pltpu.bitcast(ref[...], I32)
        acc = None
        for r in range(b.shape[0] // 8):
            for c in range(b.shape[1] // 128):
                v = b[r * 8:(r + 1) * 8, c * 128:(c + 1) * 128]
                acc = v if acc is None else acc | v
        return never(acc)

    def pq_norm(t, after=None):
        if DELAY[0] == ("p", t):
            after = delay(g_v[:, 0:T], DELAY[1]) | (after if after is not None else 0)
        pq = _ldb(pqT, 0, D, t * T, T).astype(F32)
        den = jnp.sum((pq * z_v[...]).reshape(H, DH, T), axis=1, keepdims=True) + 1e-6
        r = pl.reciprocal(den, approx=True)
        r = r * (2.0 - den * r)
        grow = g_v[0:1, t * T:(t + 1) * T]
        if after is not None:
            grow = jnp.where(after > 0, 0.0, grow)
        inv = grow.reshape(1, 1, T) * r
        _stb(pqT, 0, t * T, (pq.reshape(H, DH, T) * inv).reshape(D, T).astype(BF))

    def tile_mm(t):
        sl = slice(t * T, (t + 1) * T)
        if "ay" in FINMODE:
            a = _dot(_ldb(mT, 0, D, 0, D), _ldb(pqT, 0, D, t * T, T))
            y = _dot(_ldb(uu, 0, D, 0, F), w2_v[:, sl])
        else:
            y = _dot(_ldb(uu, 0, D, 0, F), w2_v[:, sl])
            a = _dot(_ldb(mT, 0, D, 0, D), _ldb(pqT, 0, D, t * T, T))
        return y, a

    def tile_out(t, y, a):
        sl = slice(t * T, (t + 1) * T)
        y = y + b2_v[pl.ds(t * T, T)].astype(F32).reshape(1, T)
        omg = 1.0 - g_v[:, sl]
        oT = a + (y.reshape(D // 8, 8, T) * omg[None]).reshape(D, T)
        if OUTM == "f32b":
            for m in range(4):
                outs[t][:, m * T:(m + 1) * T] = oT[m * T:(m + 1) * T].T.astype(BF)
        elif OUTM == "f32":
            outs[t][...] = oT.T.astype(BF)
        else:
            outs[t][...] = oT.astype(BF).T
        c_o[t].start()

    def anchor(k, v):
        if ANCH is True or k in ANCH:
            ANC[k][16:32, :] = v[AROW[k]:AROW[k] + 16, 0:T]

    with SC('p1'):
        first = {t0: name for name, t0, n in XS}
        def k_dot(t0, n, m):
            return _dot(x_v[t0 * T:(t0 + n) * T, :], wqkv_v[0:D, D + m * 128:D + (m + 1) * 128])

        def k_fin(t0, m, k):
            v = _phi(k).astype(BF).T
            _stb(pkT, m * 128, t0 * T, v)
            return v

        def g_rows(r0, r1, n0, n1):
            G_v[r0:r1, n0:n1] = _dot(_ldb(pkT, r0, r1 - r0, 0, CH), x_v[0:CH, n0:n1])

        g0_done = False
        if START == "nat4":
            wait("x03")
            vk = {}
            for t in range(4):
                x_transpose(t)
            for m in range(4):
                wait(f"k{m}")
                kk = k_dot(0, 4, m)
                if m == 3 and GA:
                    g_rows(0, GA, 0, GS)
                vk[m] = k_fin(0, m, kk)
            anchor(1, vk[QT])
            if TKPOS == "a":
                w_transpose(wT, 0, 1)
            if GA:
                wait("q")
                g_rows(GA, D, 0, GS)
                g0_done = True
        elif START == "nat22":
            wait("x01")
            x_transpose(0); x_transpose(1)
            wait("k0")
            k_fin(0, 0, k_dot(0, 2, 0))
            wait("k1")
            k_fin(0, 1, k_dot(0, 2, 1))
            wait("x23")
            x_transpose(2); x_transpose(3)
            k_fin(2, 0, k_dot(2, 2, 0))
            k_fin(2, 1, k_dot(2, 2, 1))
            wait("k2")
            k_fin(0, 2, k_dot(0, 4, 2))
            wait("k3")
            vv = k_fin(0, 3, k_dot(0, 4, 3))
            anchor(1, vv)
        else:
            wait("x0")
            wait("wk")
            w_transpose(wT, 0, 1)
            x_transpose(0)
            vk = {0: k_proj(0)}
            for t in range(1, 4):
                if t in first:
                    wait(first[t])
                x_transpose(t)
                vk[t] = k_proj(t)
            anchor(1, vk[QT])
        if not g0_done:
            wait("q")
            g_acc(0, 0, GS)
        if START in ("nat4", "nat22") and TKPOS == "b":
            w_transpose(wT, 0, 1)
        w_transpose(wT, D, 0)
        if VGATE:
            gwc_v[...] = jnp.broadcast_to(gw_v[...].astype(F32).reshape(1, D), (T, D)).T
        else:
            _stb(wT, 2 * D, 0, jnp.broadcast_to(gw_v[...].astype(F32).reshape(1, D), (16, D)).astype(BF))
        for t in range(4):
            layer_norm(t)
            q_proj(t)
        if 4 in first:
            wait(first[4])
        if GS < D:
            g_acc(0, GS, D)
        for c in range(1, 4):
            if c > 1 and 4 * c in first:
                wait(first[4 * c])
            for t in range(4 * c, 4 * c + 4):
                x_transpose(t)
            for t in range(4 * c, 4 * c + 4):
                layer_norm(t)
                v = kq_proj(t, direct=(t in DIRECT))
            if c < 3:
                g_acc(c)
        anchor(3, v)

    with SC('u'):
        wait("u" if "u" in grp else "us")
        w_transpose(wvT, 0, 2)
        for m in range(D // 128):
            _stb(woT, m * 128, 0, wo_v[:, m * 128:(m + 1) * 128].T)
        g_acc(3)
        if ZPOS == "a":
            z_done = z_sum()
        u_proj(0)
        kvs = kv_blocks()
        u_proj(1)
        m_matrix(kvs)
        if ZPOS == "b":
            z_done = z_sum()
        for j in range(2, F // UN):
            if j == UPOS:
                anchor(4, v)
                wait("y")
            v = u_proj(j, z_done if j == ZDEP else None)

    with SC('fin'):
        if "pipe" in FINMODE:
            prev = None
            for t in range(NTILE):
                pq_norm(t, out_done(outs[t - 2]) if t > 1 else None)
                cur = tile_mm(t)
                if prev is not None:
                    tile_out(t - 1, *prev)
                prev = cur
            tile_out(NTILE - 1, *prev)
        elif "lag2" in FINMODE:
            for t in range(NTILE):
                pq_norm(t, out_done(outs[t - 2]) if t > 1 else None)
                tile_out(t, *tile_mm(t))
        else:
            for t in range(NTILE):
                pq_norm(t, out_done(outs[t - 1]) if t > 0 else None)
                tile_out(t, *tile_mm(t))
    with SC('tail'):
        for c in c_o:
            c.wait()


def make(flags={'XLA_TPU_RESCHEDULE_DMA_DONES': True}, semchk=True, anch=True, arow=(0, 0, 0, 0, 0), scopes=False, xs=(('xd', 4, 4), ('xe', 8, 8)),
         order='x03,k0,k1,k2,k3,q,xd,xe,us,w1_2,w1_4,y', qt=2, gs=384, start='nat4', vgate=False, delay=(None, 0), late={}, zdep=2, zpos='a', zr=64, ldep=0, w1s=(0, 2, 4, 7), outm='bf', direct=(4,), ga=0, tkpos='b', upos=6, finmode='base', x0pos='early'):
    global FINMODE, X0POS, SC, XS, ORDER, QT, GS, START, GA, TKPOS, DIRECT, OUTM, VGATE, EX
    XS, ORDER, QT, GS, START, GA, TKPOS, DIRECT, OUTM = xs, order, qt, gs, start, ga, tkpos, direct, outm
    VGATE, EX = vgate, (0 if vgate else 16)
    global W1S, LDEP, ZR, ZDEP, ZPOS, LATE, DELAY
    DELAY = delay
    LATE = late
    ZR, ZDEP, ZPOS = zr, zdep, zpos
    W1S = w1s
    LDEP = ldep
    import contextlib
    SC = (lambda n: jax.named_scope(n)) if scopes else (lambda n: contextlib.nullcontext())
    FINMODE = finmode
    X0POS = x0pos
    global ANCH, AROW, UPOS
    ANCH = anch
    AROW = arow
    UPOS = upos
    @jax.jit
    def fn(A_x, A_wqkv, A_wo, B_x, B_w1, B_b1, B_w2, B_b2, gate_w):
        del B_x
        any_spec = pl.BlockSpec(memory_space=pl.ANY)
        return pl.pallas_call(
            _kernel,
            out_shape=jax.ShapeDtypeStruct((1, S, D), BF),
            in_specs=[any_spec] * 8,
            out_specs=any_spec,
            scratch_shapes=[
                pltpu.VMEM((S, D), BF),
                pltpu.VMEM((D, 3 * D), BF),
                pltpu.VMEM((D, D), BF),
                pltpu.VMEM((S, F), BF),
                pltpu.VMEM((F, S), BF),
                pltpu.VMEM((F,), BF),
                pltpu.VMEM((S,), BF),
                pltpu.VMEM((D,), BF),
                pltpu.VMEM((D + 8, D), U32),
                pltpu.VMEM((D // 2, D), U32),
                pltpu.VMEM((D // 2, D), U32),
                pltpu.VMEM((D // 2, S), U32),
                pltpu.VMEM((D // 2, S), U32),
                pltpu.VMEM((D // 2, S), U32),
                pltpu.VMEM((D // 2, S), U32),
                pltpu.VMEM((D // 2, F), U32),
                pltpu.VMEM((D // 2, D), U32),
                pltpu.VMEM((8, S), F32),
                pltpu.VMEM((D, D), F32),
                pltpu.VMEM((D, T), F32),
                pltpu.VMEM((D, T), F32),
                pltpu.SemaphoreType.DMA((1 + len(order.split(',')),)),
            ] + [pltpu.VMEM((32, T), BF)] * 5 + [pltpu.VMEM((T, D), BF)] * NTILE,
            compiler_params=pltpu.CompilerParams(vmem_limit_bytes=100 * 1024 * 1024, flags=flags,
                                                 disable_semaphore_checks=not semchk),
        )(A_x, A_wqkv, A_wo, B_w1, B_b1, B_w2, B_b2, gate_w)

    return fn


_fn = make()


def pallas_gated_mix__linear_attn_block__mixer_token_mlp__prompt_kernel(A_x, A_wqkv, A_wo, B_x, B_w1, B_b1, B_w2, B_b2, gate_w):
    return _fn(A_x, A_wqkv, A_wo, B_x, B_w1, B_b1, B_w2, B_b2, gate_w)
```

```python
import jax
import jax.numpy as jnp
from jax import lax
from jax.experimental import pallas as pl
from jax.experimental.pallas import tpu as pltpu

S, D, F, H, DH = 2048, 512, 1792, 32, 16
T = 128
NTILE = S // T
CH = 512
UN = 256
BF, F32, U32, I32 = jnp.bfloat16, jnp.float32, jnp.uint32, jnp.int32
NN = (((1,), (0,)), ((), ()))
NT = (((1,), (1,)), ((), ()))
W1_CUTS = (0, 2, 4, 7)
N_DMA_GROUPS = 12


def _dot(a, b, dims=NN):
    return lax.dot_general(a, b, dims, preferred_element_type=F32)


def _phi(t):
    return jnp.where(t > 0, t + 1.0, jnp.exp(t)) + 1e-6


def _gelu(x):
    return 0.5 * x * (1.0 + jnp.tanh(0.7978845608028654 * (x + 0.044715 * (x * x * x))))


def _ldb(ref, r0, rows, c0, cols):
    return pltpu.bitcast(ref[r0 // 2:(r0 + rows) // 2, c0:c0 + cols], BF)


def _stb(ref, r0, c0, val):
    rows, cols = val.shape
    ref[r0 // 2:(r0 + rows) // 2, c0:c0 + cols] = pltpu.bitcast(val, U32)


def _kernel(ax_hbm, wqkv_hbm, wo_hbm, w1_hbm, b1_hbm, w2_hbm, b2_hbm, gw_hbm, o_hbm,
            x_v, wqkv_v, wo_v, w1_v, w2_v, b1_v, b2_v, gw_v,
            wT, wvT, woT, xT, hT, pkT, pqT, uu, mT, g_v, G_v, z_v, sems, *rest):
    anc, outs = rest[:3], rest[3:]

    def cp(src, dst, i):
        return pltpu.make_async_copy(src, dst, sems.at[i])

    def x_cp(t0, n, i):
        return cp(ax_hbm.at[0, pl.ds(t0 * T, n * T)], x_v.at[pl.ds(t0 * T, n * T)], i)

    def col_cp(src, dst, c0, n, i):
        return cp(src.at[:, pl.ds(c0, n)], dst.at[:, pl.ds(c0, n)], i)

    def anc_cp(k, i):
        return cp(wo_hbm.at[pl.ds(0, 16), pl.ds(0, T)], anc[k].at[pl.ds(0, 16)], i)

    groups = [[x_cp(0, 4, 0)]]
    groups += [[col_cp(wqkv_hbm, wqkv_v, D + m * 128, 128, 1 + m)] for m in range(4)]
    groups += [[col_cp(wqkv_hbm, wqkv_v, 0, D, 5), cp(gw_hbm, gw_v, 5), anc_cp(0, 5)]]
    groups += [[x_cp(4, 4, 6)], [x_cp(8, 8, 7)]]
    groups += [[col_cp(wqkv_hbm, wqkv_v, 2 * D, D, 8), cp(wo_hbm, wo_v, 8), cp(b1_hbm, b1_v, 8),
                col_cp(w1_hbm, w1_v, 0, W1_CUTS[1] * UN, 8), anc_cp(1, 8)]]
    groups += [[col_cp(w1_hbm, w1_v, a * UN, (b - a) * UN, 9 + i)]
               for i, (a, b) in enumerate(zip(W1_CUTS[1:-1], W1_CUTS[2:]))]
    groups += [[cp(b2_hbm, b2_v, 11), cp(w2_hbm, w2_v, 11), anc_cp(2, 11)]]
    g_x0, g_k0, g_q, g_x1, g_x2, g_u, g_w1, g_y = 0, 1, 5, 6, 7, 8, 9, 11
    c_o = [cp(outs[j], o_hbm.at[0, pl.ds(j * T, T)], N_DMA_GROUPS) for j in range(NTILE)]
    for grp in groups:
        for c in grp:
            c.start()

    def wait(i):
        for c in groups[i]:
            c.wait()

    def anchor(k, v):
        anc[k][16:32, :] = v[0:16, 0:T]

    def w_transpose(dst, r0, j):
        for m in range(D // 128):
            _stb(dst, r0 + m * 128, 0, wqkv_v[:, j * D + m * 128:j * D + (m + 1) * 128].T)

    def x_tile(t):
        return x_v[t * T:(t + 1) * T, :]

    def x_transpose(t):
        _stb(xT, 0, t * T, x_tile(t).T)

    def proj(t, r0, rows, direct):
        w = _ldb(wT, r0, rows, 0, D)
        if direct:
            return _dot(w, x_tile(t), NT)
        return _dot(w, _ldb(xT, 0, D, t * T, T))

    def q_post(t, qT):
        v = _phi(qT[0:D]).astype(BF)
        _stb(pqT, 0, t * T, v)
        g_v[:, t * T:(t + 1) * T] = jax.nn.sigmoid(qT[D:D + 8])
        return v

    def k_first(m):
        k = _dot(x_v[0:CH, :], wqkv_v[:, D + m * 128:D + (m + 1) * 128])
        v = _phi(k).astype(BF).T
        _stb(pkT, m * 128, 0, v)
        return v

    def q_proj(t):
        return q_post(t, proj(t, D, D + 16, False))

    def kq_proj(t, direct):
        r = proj(t, 0, 2 * D + 16, direct)
        _stb(pkT, 0, t * T, _phi(r[0:D]).astype(BF))
        return q_post(t, r[D:2 * D + 16])

    def layer_norm(t):
        b = _ldb(xT, 0, D, t * T, T).astype(F32)
        d = b - jnp.mean(b, axis=0, keepdims=True)
        var = jnp.mean(d * d, axis=0, keepdims=True)
        _stb(hT, 0, t * T, (d * lax.rsqrt(var + 1e-5)).astype(BF))

    def g_acc(c, n0=0, n1=D):
        Gc = _dot(_ldb(pkT, 0, D, c * CH, CH), x_v[c * CH:(c + 1) * CH, n0:n1])
        if c == 0:
            G_v[:, n0:n1] = Gc
        else:
            G_v[:, n0:n1] += Gc

    def never(bits):
        return jnp.minimum(bits[0:1, :], 0)

    def z_sum():
        acc = _ldb(pkT, 0, D, 0, T).astype(F32)
        for t in range(1, NTILE):
            acc = acc + _ldb(pkT, 0, D, t * T, T).astype(F32)
        zb = jnp.broadcast_to(jnp.sum(acc, axis=1, keepdims=True), (D, T))
        z_v[...] = zb
        zi = pltpu.bitcast(zb, I32)
        a = zi[0:8]
        for r in range(1, D // 8):
            a = a | zi[r * 8:(r + 1) * 8]
        return never(a)

    def u_proj(j, after=None):
        acc = _dot(_ldb(hT, 0, D, 0, S), w1_v[:, j * UN:(j + 1) * UN])
        bias = b1_v[pl.ds(j * UN, UN)].astype(F32).reshape(1, UN)
        if after is not None:
            bias = jnp.where(jnp.concatenate([after] * (UN // T), axis=1) > 0, 0.0, bias)
        v = _gelu(acc + bias).astype(BF)
        _stb(uu, 0, j * UN, v)
        return v

    def kv_blocks():
        ri = lax.broadcasted_iota(I32, (128, 128), 0) // DH
        ci = lax.broadcasted_iota(I32, (128, 128), 1) // DH
        out = []
        for gp in range(D // 128):
            kvT = _dot(_ldb(wvT, gp * 128, 128, 0, D), G_v[gp * 128:(gp + 1) * 128, :].astype(BF), NT)
            out.append(jnp.where(ri == ci, kvT, 0.0).astype(BF))
        return out

    def m_matrix(kvs):
        for gp in range(D // 128):
            _stb(mT, 0, gp * 128, _dot(_ldb(woT, 0, D, gp * 128, 128), kvs[gp]).astype(BF))

    def out_done(ref):
        b = pltpu.bitcast(ref[...], I32)
        acc = None
        for r in range(b.shape[0] // 8):
            for c in range(b.shape[1] // 128):
                v = b[r * 8:(r + 1) * 8, c * 128:(c + 1) * 128]
                acc = v if acc is None else acc | v
        return never(acc)

    def pq_norm(t, after=None):
        pq = _ldb(pqT, 0, D, t * T, T).astype(F32)
        den = jnp.sum((pq * z_v[...]).reshape(H, DH, T), axis=1, keepdims=True) + 1e-6
        r = pl.reciprocal(den, approx=True)
        r = r * (2.0 - den * r)
        grow = g_v[0:1, t * T:(t + 1) * T]
        if after is not None:
            grow = jnp.where(after > 0, 0.0, grow)
        inv = grow.reshape(1, 1, T) * r
        _stb(pqT, 0, t * T, (pq.reshape(H, DH, T) * inv).reshape(D, T).astype(BF))

    def out_tile(t):
        sl = slice(t * T, (t + 1) * T)
        y = _dot(_ldb(uu, 0, D, 0, F), w2_v[:, sl])
        a = _dot(_ldb(mT, 0, D, 0, D), _ldb(pqT, 0, D, t * T, T))
        y = y + b2_v[pl.ds(t * T, T)].astype(F32).reshape(1, T)
        omg = 1.0 - g_v[:, sl]
        oT = a + (y.reshape(D // 8, 8, T) * omg[None]).reshape(D, T)
        outs[t][...] = oT.astype(BF).T
        c_o[t].start()

    wait(g_x0)
    for t in range(4):
        x_transpose(t)
    vk = []
    for m in range(4):
        wait(g_k0 + m)
        vk.append(k_first(m))
    anchor(0, vk[2])
    wait(g_q)
    g_acc(0, 0, 384)
    w_transpose(wT, 0, 1)
    w_transpose(wT, D, 0)
    _stb(wT, 2 * D, 0, jnp.broadcast_to(gw_v[...].astype(F32).reshape(1, D), (16, D)).astype(BF))
    for t in range(4):
        layer_norm(t)
        q_proj(t)

    wait(g_x1)
    g_acc(0, 384, D)
    for c in range(1, 4):
        if c == 2:
            wait(g_x2)
        for t in range(4 * c, 4 * c + 4):
            x_transpose(t)
        for t in range(4 * c, 4 * c + 4):
            layer_norm(t)
            v = kq_proj(t, direct=(t == 4))
        if c < 3:
            g_acc(c)
    anchor(1, v)

    wait(g_u)
    w_transpose(wvT, 0, 2)
    for m in range(D // 128):
        _stb(woT, m * 128, 0, wo_v[:, m * 128:(m + 1) * 128].T)
    g_acc(3)
    z_done = z_sum()
    kvs = None
    for j in range(F // UN):
        if j in W1_CUTS[1:-1]:
            wait(g_w1 + W1_CUTS.index(j) - 1)
        if j == F // UN - 1:
            anchor(2, v)
            wait(g_y)
        v = u_proj(j, z_done if j == 2 else None)
        if j == 0:
            kvs = kv_blocks()
        if j == 1:
            m_matrix(kvs)

    for t in range(NTILE):
        pq_norm(t, out_done(outs[t - 1]) if t > 0 else None)
        out_tile(t)
    for c in c_o:
        c.wait()


def make():
    @jax.jit
    def fn(A_x, A_wqkv, A_wo, B_x, B_w1, B_b1, B_w2, B_b2, gate_w):
        del B_x
        any_spec = pl.BlockSpec(memory_space=pl.ANY)
        return pl.pallas_call(
            _kernel,
            out_shape=jax.ShapeDtypeStruct((1, S, D), BF),
            in_specs=[any_spec] * 8,
            out_specs=any_spec,
            scratch_shapes=[
                pltpu.VMEM((S, D), BF),
                pltpu.VMEM((D, 3 * D), BF),
                pltpu.VMEM((D, D), BF),
                pltpu.VMEM((S, F), BF),
                pltpu.VMEM((F, S), BF),
                pltpu.VMEM((F,), BF),
                pltpu.VMEM((S,), BF),
                pltpu.VMEM((D,), BF),
                pltpu.VMEM((D + 8, D), U32),
                pltpu.VMEM((D // 2, D), U32),
                pltpu.VMEM((D // 2, D), U32),
                pltpu.VMEM((D // 2, S), U32),
                pltpu.VMEM((D // 2, S), U32),
                pltpu.VMEM((D // 2, S), U32),
                pltpu.VMEM((D // 2, S), U32),
                pltpu.VMEM((D // 2, F), U32),
                pltpu.VMEM((D // 2, D), U32),
                pltpu.VMEM((8, S), F32),
                pltpu.VMEM((D, D), F32),
                pltpu.VMEM((D, T), F32),
                pltpu.SemaphoreType.DMA((N_DMA_GROUPS + 1,)),
            ] + [pltpu.VMEM((32, T), BF)] * 3
              + [pltpu.VMEM((T, D), BF)] * NTILE,
            compiler_params=pltpu.CompilerParams(
                vmem_limit_bytes=100 * 1024 * 1024,
                flags={"XLA_TPU_RESCHEDULE_DMA_DONES": True},
            ),
        )(A_x, A_wqkv, A_wo, B_w1, B_b1, B_w2, B_b2, gate_w)

    return fn


_fn = make()


def pallas_gated_mix__linear_attn_block__mixer_token_mlp__prompt_kernel(A_x, A_wqkv, A_wo, B_x, B_w1, B_b1, B_w2, B_b2, gate_w):
    return _fn(A_x, A_wqkv, A_wo, B_x, B_w1, B_b1, B_w2, B_b2, gate_w)
```

```python
import jax
import jax.numpy as jnp
from jax import lax
from jax.experimental import pallas as pl
from jax.experimental.pallas import tpu as pltpu

S, D, F, H, DH = 2048, 512, 1792, 32, 16
T = 128
NTILE = S // T
CH = 512
UN = 256
BF, F32, U32, I32 = jnp.bfloat16, jnp.float32, jnp.uint32, jnp.int32
NN = (((1,), (0,)), ((), ()))
NT = (((1,), (1,)), ((), ()))
W1_CUTS = (0, 2, 4, 7)
N_DMA_GROUPS = 14


def _dot(a, b, dims=NN):
    return lax.dot_general(a, b, dims, preferred_element_type=F32)


def _phi(t):
    return jnp.where(t > 0, t + 1.0, jnp.exp(t)) + 1e-6


def _gelu(x):
    return 0.5 * x * (1.0 + jnp.tanh(0.7978845608028654 * (x + 0.044715 * (x * x * x))))


def _ldb(ref, r0, rows, c0, cols):
    return pltpu.bitcast(ref[r0 // 2:(r0 + rows) // 2, c0:c0 + cols], BF)


def _stb(ref, r0, c0, val):
    rows, cols = val.shape
    ref[r0 // 2:(r0 + rows) // 2, c0:c0 + cols] = pltpu.bitcast(val, U32)


def _kernel(ax_hbm, wqkv_hbm, wo_hbm, w1_hbm, b1_hbm, w2_hbm, b2_hbm, gw_hbm, o_hbm,
            x_v, wqkv_v, wo_v, w1_v, w2_v, b1_v, b2_v, gw_v,
            wT, wvT, woT, xT, hT, pkT, pqT, uu, mT, g_v, G_v, z_v, st_v, sems, *rest):
    anc, outs = rest[:3], rest[3:]

    def cp(src, dst, i):
        return pltpu.make_async_copy(src, dst, sems.at[i])

    def x_cp(t0, n, i):
        return cp(ax_hbm.at[0, pl.ds(t0 * T, n * T)], x_v.at[pl.ds(t0 * T, n * T)], i)

    def col_cp(src, dst, c0, n, i):
        return cp(src.at[:, pl.ds(c0, n)], dst.at[:, pl.ds(c0, n)], i)

    def anc_cp(k, i):
        return cp(wo_hbm.at[pl.ds(0, 16), pl.ds(0, T)], anc[k].at[pl.ds(0, 16)], i)

    head = [("x", 0, 2), ("k", 0), ("k", 1), ("x", 2, 1), ("k", 2), ("x", 3, 1), ("k", 3)]
    groups = [[x_cp(h[1], h[2], i) if h[0] == "x" else col_cp(wqkv_hbm, wqkv_v, D + h[1] * 128, 128, i)]
              for i, h in enumerate(head)]
    g_q, g_x1, g_x2, g_u, g_w1, g_y = 7, 8, 9, 10, 11, 13
    groups += [[col_cp(wqkv_hbm, wqkv_v, 0, D, g_q), cp(gw_hbm, gw_v, g_q), anc_cp(0, g_q)]]
    groups += [[x_cp(4, 4, g_x1)], [x_cp(8, 8, g_x2)]]
    groups += [[col_cp(wqkv_hbm, wqkv_v, 2 * D, D, g_u), cp(wo_hbm, wo_v, g_u), cp(b1_hbm, b1_v, g_u),
                col_cp(w1_hbm, w1_v, 0, W1_CUTS[1] * UN, g_u), anc_cp(1, g_u)]]
    groups += [[col_cp(w1_hbm, w1_v, a * UN, (b - a) * UN, g_w1 + i)]
               for i, (a, b) in enumerate(zip(W1_CUTS[1:-1], W1_CUTS[2:]))]
    groups += [[cp(b2_hbm, b2_v, g_y), cp(w2_hbm, w2_v, g_y), anc_cp(2, g_y)]]
    assert len(groups) == N_DMA_GROUPS
    c_o = [cp(outs[j], o_hbm.at[0, pl.ds(j * T, T)], N_DMA_GROUPS) for j in range(NTILE)]
    for grp in groups:
        for c in grp:
            c.start()

    def wait(i):
        for c in groups[i]:
            c.wait()

    def anchor(k, v):
        anc[k][16:32, :] = v[0:16, 0:T]

    def w_transpose(dst, r0, j):
        for m in range(D // 128):
            _stb(dst, r0 + m * 128, 0, wqkv_v[:, j * D + m * 128:j * D + (m + 1) * 128].T)

    def x_tile(t):
        return x_v[t * T:(t + 1) * T, :]

    def x_transpose(t):
        _stb(xT, 0, t * T, x_tile(t).T)

    def proj(t, r0, rows):
        return _dot(_ldb(wT, r0, rows, 0, D), _ldb(xT, 0, D, t * T, T))

    def q_post(t, qT):
        v = _phi(qT[0:D]).astype(BF)
        _stb(pqT, 0, t * T, v)
        g_v[:, t * T:(t + 1) * T] = jax.nn.sigmoid(qT[D:D + 8])
        return v

    def k_first(t0, n, m):
        k = _dot(x_v[t0 * T:(t0 + n) * T, :], wqkv_v[:, D + m * 128:D + (m + 1) * 128])
        v = _phi(k).astype(BF).T
        _stb(pkT, m * 128, t0 * T, v)
        return v

    def q_proj(t):
        return q_post(t, proj(t, D, D + 16))

    def kq_proj(t):
        r = proj(t, 0, 2 * D + 16)
        _stb(pkT, 0, t * T, _phi(r[0:D]).astype(BF))
        return q_post(t, r[D:2 * D + 16])

    def layer_norm(t):
        m = jnp.mean(_ldb(xT, 0, D, t * T, T).astype(F32), axis=0, keepdims=True)
        st_v[0:1, :] = m
        d = _ldb(xT, 0, D, t * T, T).astype(F32) - m
        r = lax.rsqrt(jnp.mean(d * d, axis=0, keepdims=True) + 1e-5)
        st_v[1:2, :] = r
        _stb(hT, 0, t * T, ((_ldb(xT, 0, D, t * T, T).astype(F32) - m) * r).astype(BF))

    def g_acc(c):
        Gc = _dot(_ldb(pkT, 0, D, c * CH, CH), x_v[c * CH:(c + 1) * CH, :])
        if c == 0:
            G_v[...] = Gc
        else:
            G_v[...] += Gc

    def never(bits):
        return jnp.minimum(bits[0:1, :], 0)

    def z_sum():
        acc = _ldb(pkT, 0, D, 0, T).astype(F32)
        for t in range(1, NTILE):
            acc = acc + _ldb(pkT, 0, D, t * T, T).astype(F32)
        zb = jnp.broadcast_to(jnp.sum(acc, axis=1, keepdims=True), (D, T))
        z_v[...] = zb
        zi = pltpu.bitcast(zb, I32)
        a = zi[0:8]
        for r in range(1, D // 8):
            a = a | zi[r * 8:(r + 1) * 8]
        return never(a)

    def u_proj(j, after=None):
        acc = _dot(_ldb(hT, 0, D, 0, S), w1_v[:, j * UN:(j + 1) * UN])
        bias = b1_v[pl.ds(j * UN, UN)].astype(F32).reshape(1, UN)
        if after is not None:
            bias = jnp.where(jnp.concatenate([after] * (UN // T), axis=1) > 0, 0.0, bias)
        v = _gelu(acc + bias).astype(BF)
        _stb(uu, 0, j * UN, v)
        return v

    def kv_blocks():
        ri = lax.broadcasted_iota(I32, (128, 128), 0) // DH
        ci = lax.broadcasted_iota(I32, (128, 128), 1) // DH
        out = []
        for gp in range(D // 128):
            kvT = _dot(_ldb(wvT, gp * 128, 128, 0, D), G_v[gp * 128:(gp + 1) * 128, :].astype(BF), NT)
            out.append(jnp.where(ri == ci, kvT, 0.0).astype(BF))
        return out

    def m_matrix(kvs):
        for gp in range(D // 128):
            _stb(mT, 0, gp * 128, _dot(_ldb(woT, 0, D, gp * 128, 128), kvs[gp]).astype(BF))

    def out_done(ref):
        b = pltpu.bitcast(ref[...], I32)
        acc = None
        for r in range(b.shape[0] // 8):
            for c in range(b.shape[1] // 128):
                v = b[r * 8:(r + 1) * 8, c * 128:(c + 1) * 128]
                acc = v if acc is None else acc | v
        return never(acc)

    def pq_norm(t, after=None):
        pq = _ldb(pqT, 0, D, t * T, T).astype(F32)
        den = jnp.sum((pq * z_v[...]).reshape(H, DH, T), axis=1, keepdims=True) + 1e-6
        r = pl.reciprocal(den, approx=True)
        r = r * (2.0 - den * r)
        grow = g_v[0:1, t * T:(t + 1) * T]
        if after is not None:
            grow = jnp.where(after > 0, 0.0, grow)
        inv = grow.reshape(1, 1, T) * r
        _stb(pqT, 0, t * T, (pq.reshape(H, DH, T) * inv).reshape(D, T).astype(BF))

    def out_tile(t):
        sl = slice(t * T, (t + 1) * T)
        y = _dot(_ldb(uu, 0, D, 0, F), w2_v[:, sl])
        a = _dot(_ldb(mT, 0, D, 0, D), _ldb(pqT, 0, D, t * T, T))
        y = y + b2_v[pl.ds(t * T, T)].astype(F32).reshape(1, T)
        omg = 1.0 - g_v[:, sl]
        oT = a + (y.reshape(D // 8, 8, T) * omg[None]).reshape(D, T)
        outs[t][...] = oT.astype(BF).T
        c_o[t].start()

    n_tiles, blocks, v = 0, [], None
    for i, h in enumerate(head):
        wait(i)
        if h[0] == "x":
            for t in range(h[1], h[1] + h[2]):
                x_transpose(t)
            for m in blocks:
                v = k_first(h[1], h[2], m)
            n_tiles = h[1] + h[2]
        else:
            blocks.append(h[1])
            v = k_first(0, n_tiles, h[1])
    anchor(0, v)
    wait(g_q)
    g_acc(0)
    w_transpose(wT, 0, 1)
    w_transpose(wT, D, 0)
    _stb(wT, 2 * D, 0, jnp.broadcast_to(gw_v[...].astype(F32).reshape(1, D), (16, D)).astype(BF))
    for t in range(4):
        layer_norm(t)
        q_proj(t)

    wait(g_x1)
    for c in range(1, 4):
        if c == 2:
            wait(g_x2)
        for t in range(4 * c, 4 * c + 4):
            x_transpose(t)
        for t in range(4 * c, 4 * c + 4):
            layer_norm(t)
            v = kq_proj(t)
        if c < 3:
            g_acc(c)
    anchor(1, v)

    wait(g_u)
    w_transpose(wvT, 0, 2)
    for m in range(D // 128):
        _stb(woT, m * 128, 0, wo_v[:, m * 128:(m + 1) * 128].T)
    g_acc(3)
    z_done = z_sum()
    kvs = None
    for j in range(F // UN):
        if j in W1_CUTS[1:-1]:
            wait(g_w1 + W1_CUTS.index(j) - 1)
        if j == F // UN - 1:
            anchor(2, v)
            wait(g_y)
        v = u_proj(j, z_done if j == 2 else None)
        if j == 0:
            kvs = kv_blocks()
        if j == 1:
            m_matrix(kvs)

    for t in range(NTILE):
        pq_norm(t, out_done(outs[t - 1]) if t > 0 else None)
        out_tile(t)
    for c in c_o:
        c.wait()


def make():
    @jax.jit
    def fn(A_x, A_wqkv, A_wo, B_x, B_w1, B_b1, B_w2, B_b2, gate_w):
        del B_x
        any_spec = pl.BlockSpec(memory_space=pl.ANY)
        return pl.pallas_call(
            _kernel,
            out_shape=jax.ShapeDtypeStruct((1, S, D), BF),
            in_specs=[any_spec] * 8,
            out_specs=any_spec,
            scratch_shapes=[
                pltpu.VMEM((S, D), BF),
                pltpu.VMEM((D, 3 * D), BF),
                pltpu.VMEM((D, D), BF),
                pltpu.VMEM((S, F), BF),
                pltpu.VMEM((F, S), BF),
                pltpu.VMEM((F,), BF),
                pltpu.VMEM((S,), BF),
                pltpu.VMEM((D,), BF),
                pltpu.VMEM((D + 8, D), U32),
                pltpu.VMEM((D // 2, D), U32),
                pltpu.VMEM((D // 2, D), U32),
                pltpu.VMEM((D // 2, S), U32),
                pltpu.VMEM((D // 2, S), U32),
                pltpu.VMEM((D // 2, S), U32),
                pltpu.VMEM((D // 2, S), U32),
                pltpu.VMEM((D // 2, F), U32),
                pltpu.VMEM((D // 2, D), U32),
                pltpu.VMEM((8, S), F32),
                pltpu.VMEM((D, D), F32),
                pltpu.VMEM((D, T), F32),
                pltpu.VMEM((8, T), F32),
                pltpu.SemaphoreType.DMA((N_DMA_GROUPS + 1,)),
            ] + [pltpu.VMEM((32, T), BF)] * 3
              + [pltpu.VMEM((T, D), BF)] * NTILE,
            compiler_params=pltpu.CompilerParams(
                vmem_limit_bytes=100 * 1024 * 1024,
                flags={"XLA_TPU_RESCHEDULE_DMA_DONES": True},
            ),
        )(A_x, A_wqkv, A_wo, B_w1, B_b1, B_w2, B_b2, gate_w)

    return fn


_fn = make()


def pallas_gated_mix__linear_attn_block__mixer_token_mlp__prompt_kernel(A_x, A_wqkv, A_wo, B_x, B_w1, B_b1, B_w2, B_b2, gate_w):
    return _fn(A_x, A_wqkv, A_wo, B_x, B_w1, B_b1, B_w2, B_b2, gate_w)
```

```python
import jax
import jax.numpy as jnp
from jax import lax
from jax.experimental import pallas as pl
from jax.experimental.pallas import tpu as pltpu

S, D, F, H, DH = 2048, 512, 1792, 32, 16
T = 128
NTILE = S // T
CH = 512
UN = 256
BF, F32, U32, I32 = jnp.bfloat16, jnp.float32, jnp.uint32, jnp.int32
NN = (((1,), (0,)), ((), ()))
NT = (((1,), (1,)), ((), ()))
W1_CUTS = (0, 2, 4, 7)
N_DMA_GROUPS = 14


def _dot(a, b, dims=NN):
    return lax.dot_general(a, b, dims, preferred_element_type=F32)


def _phi(t):
    return jnp.where(t > 0, t + 1.0, jnp.exp(t)) + 1e-6


def _gelu(x):
    return 0.5 * x * (1.0 + jnp.tanh(0.7978845608028654 * (x + 0.044715 * (x * x * x))))


def _ldb(ref, r0, rows, c0, cols):
    return pltpu.bitcast(ref[r0 // 2:(r0 + rows) // 2, c0:c0 + cols], BF)


def _stb(ref, r0, c0, val):
    rows, cols = val.shape
    ref[r0 // 2:(r0 + rows) // 2, c0:c0 + cols] = pltpu.bitcast(val, U32)


def _kernel(ax_hbm, wqkv_hbm, wo_hbm, w1_hbm, b1_hbm, w2_hbm, b2_hbm, gw_hbm, o_hbm,
            x_v, wqkv_v, wo_v, w1_v, w2_v, b1_v, b2_v, gw_v,
            wT, wvT, woT, xT, hT, pkT, pqT, uu, mT, g_v, G_v, z_v, st_v, sems, *rest):
    anc, outs = rest[:3], rest[3:]

    def cp(src, dst, i):
        return pltpu.make_async_copy(src, dst, sems.at[i])

    def x_cp(t0, n, i):
        return cp(ax_hbm.at[0, pl.ds(t0 * T, n * T)], x_v.at[pl.ds(t0 * T, n * T)], i)

    def col_cp(src, dst, c0, n, i):
        return cp(src.at[:, pl.ds(c0, n)], dst.at[:, pl.ds(c0, n)], i)

    def anc_cp(k, i):
        return cp(wo_hbm.at[pl.ds(0, 16), pl.ds(0, T)], anc[k].at[pl.ds(0, 16)], i)

    head = [("x", 0, 2), ("k", 0), ("k", 1), ("x", 2, 1), ("k", 2), ("x", 3, 1), ("k", 3)]
    groups = [[x_cp(h[1], h[2], i) if h[0] == "x" else col_cp(wqkv_hbm, wqkv_v, D + h[1] * 128, 128, i)]
              for i, h in enumerate(head)]
    g_q, g_x1, g_x2, g_u, g_w1, g_y = 7, 8, 9, 10, 11, 13
    groups += [[col_cp(wqkv_hbm, wqkv_v, 0, D, g_q), cp(gw_hbm, gw_v, g_q), anc_cp(0, g_q)]]
    groups += [[x_cp(4, 4, g_x1)], [x_cp(8, 8, g_x2)]]
    groups += [[col_cp(wqkv_hbm, wqkv_v, 2 * D, D, g_u), cp(wo_hbm, wo_v, g_u), cp(b1_hbm, b1_v, g_u),
                col_cp(w1_hbm, w1_v, 0, W1_CUTS[1] * UN, g_u), anc_cp(1, g_u)]]
    groups += [[col_cp(w1_hbm, w1_v, a * UN, (b - a) * UN, g_w1 + i)]
               for i, (a, b) in enumerate(zip(W1_CUTS[1:-1], W1_CUTS[2:]))]
    groups += [[cp(b2_hbm, b2_v, g_y), cp(w2_hbm, w2_v, g_y), anc_cp(2, g_y)]]
    assert len(groups) == N_DMA_GROUPS
    c_o = [cp(outs[j], o_hbm.at[0, pl.ds(j * T, T)], N_DMA_GROUPS) for j in range(NTILE)]
    for grp in groups:
        for c in grp:
            c.start()

    def wait(i):
        for c in groups[i]:
            c.wait()

    def anchor(k, v):
        anc[k][16:32, :] = v[0:16, 0:T]

    def w_transpose(dst, r0, j):
        for m in range(D // 128):
            _stb(dst, r0 + m * 128, 0, wqkv_v[:, j * D + m * 128:j * D + (m + 1) * 128].T)

    def x_tile(t):
        return x_v[t * T:(t + 1) * T, :]

    def x_transpose(t):
        _stb(xT, 0, t * T, x_tile(t).T)

    def proj(t, r0, rows):
        return _dot(_ldb(wT, r0, rows, 0, D), _ldb(xT, 0, D, t * T, T))

    def q_post(t, qT):
        v = _phi(qT[0:D]).astype(BF)
        _stb(pqT, 0, t * T, v)
        g_v[:, t * T:(t + 1) * T] = jax.nn.sigmoid(qT[D:D + 8])
        return v

    def k_first(t0, n, m):
        k = _dot(x_v[t0 * T:(t0 + n) * T, :], wqkv_v[:, D + m * 128:D + (m + 1) * 128])
        v = _phi(k).astype(BF).T
        _stb(pkT, m * 128, t0 * T, v)
        return v

    def q_proj(t):
        return q_post(t, proj(t, D, D + 16))

    def kq_proj(t):
        r = proj(t, 0, 2 * D + 16)
        _stb(pkT, 0, t * T, _phi(r[0:D]).astype(BF))
        return q_post(t, r[D:2 * D + 16])

    def layer_norm(t):
        m = jnp.mean(_ldb(xT, 0, D, t * T, T).astype(F32), axis=0, keepdims=True)
        st_v[0:1, :] = m
        d = _ldb(xT, 0, D, t * T, T).astype(F32) - m
        r = lax.rsqrt(jnp.mean(d * d, axis=0, keepdims=True) + 1e-5)
        st_v[1:2, :] = r
        _stb(hT, 0, t * T, ((_ldb(xT, 0, D, t * T, T).astype(F32) - m) * r).astype(BF))

    def g_acc(c):
        Gc = _dot(_ldb(pkT, 0, D, c * CH, CH), x_v[c * CH:(c + 1) * CH, :])
        if c == 0:
            G_v[...] = Gc
        else:
            G_v[...] += Gc

    def never(bits):
        return jnp.minimum(bits[0:1, :], 0)

    def z_sum():
        acc = _ldb(pkT, 0, D, 0, T).astype(F32)
        for t in range(1, NTILE):
            acc = acc + _ldb(pkT, 0, D, t * T, T).astype(F32)
        zb = jnp.broadcast_to(jnp.sum(acc, axis=1, keepdims=True), (D, T))
        z_v[...] = zb
        zi = pltpu.bitcast(zb, I32)
        a = zi[0:8]
        for r in range(1, D // 8):
            a = a | zi[r * 8:(r + 1) * 8]
        return never(a)

    def u_proj(j, after=None):
        acc = _dot(_ldb(hT, 0, D, 0, S), w1_v[:, j * UN:(j + 1) * UN])
        bias = b1_v[pl.ds(j * UN, UN)].astype(F32).reshape(1, UN)
        if after is not None:
            bias = jnp.where(jnp.concatenate([after] * (UN // T), axis=1) > 0, 0.0, bias)
        v = _gelu(acc + bias).astype(BF)
        _stb(uu, 0, j * UN, v)
        return v

    def kv_blocks():
        ri = lax.broadcasted_iota(I32, (128, 128), 0) // DH
        ci = lax.broadcasted_iota(I32, (128, 128), 1) // DH
        out = []
        for gp in range(D // 128):
            kvT = _dot(_ldb(wvT, gp * 128, 128, 0, D), G_v[gp * 128:(gp + 1) * 128, :].astype(BF), NT)
            out.append(jnp.where(ri == ci, kvT, 0.0).astype(BF))
        return out

    def m_matrix(kvs):
        for gp in range(D // 128):
            _stb(mT, 0, gp * 128, _dot(_ldb(woT, 0, D, gp * 128, 128), kvs[gp]).astype(BF))

    def out_done(ref):
        b = pltpu.bitcast(ref[T - 16:T, :], I32)
        acc = b[:, 0:128]
        for c in range(1, D // 128):
            acc = acc | b[:, c * 128:(c + 1) * 128]
        return never(acc)

    def pq_norm(t, after=None):
        pq = _ldb(pqT, 0, D, t * T, T).astype(F32)
        den = jnp.sum((pq * z_v[...]).reshape(H, DH, T), axis=1, keepdims=True) + 1e-6
        r = pl.reciprocal(den, approx=True)
        r = r * (2.0 - den * r)
        grow = g_v[0:1, t * T:(t + 1) * T]
        if after is not None:
            grow = jnp.where(after > 0, 0.0, grow)
        inv = grow.reshape(1, 1, T) * r
        _stb(pqT, 0, t * T, (pq.reshape(H, DH, T) * inv).reshape(D, T).astype(BF))

    def out_tile(t):
        sl = slice(t * T, (t + 1) * T)
        y = _dot(_ldb(uu, 0, D, 0, F), w2_v[:, sl])
        a = _dot(_ldb(mT, 0, D, 0, D), _ldb(pqT, 0, D, t * T, T))
        y = y + b2_v[pl.ds(t * T, T)].astype(F32).reshape(1, T)
        omg = 1.0 - g_v[:, sl]
        oT = a + (y.reshape(D // 8, 8, T) * omg[None]).reshape(D, T)
        outs[t][...] = oT.astype(BF).T
        c_o[t].start()

    n_tiles, blocks, v = 0, [], None
    for i, h in enumerate(head):
        wait(i)
        if h[0] == "x":
            for t in range(h[1], h[1] + h[2]):
                x_transpose(t)
            for m in blocks:
                v = k_first(h[1], h[2], m)
            n_tiles = h[1] + h[2]
        else:
            blocks.append(h[1])
            v = k_first(0, n_tiles, h[1])
    anchor(0, v)
    wait(g_q)
    g_acc(0)
    w_transpose(wT, 0, 1)
    w_transpose(wT, D, 0)
    _stb(wT, 2 * D, 0, jnp.broadcast_to(gw_v[...].astype(F32).reshape(1, D), (16, D)).astype(BF))
    for t in range(4):
        layer_norm(t)
        q_proj(t)

    wait(g_x1)
    for c in range(1, 4):
        if c == 2:
            wait(g_x2)
        for t in range(4 * c, 4 * c + 4):
            x_transpose(t)
        for t in range(4 * c, 4 * c + 4):
            layer_norm(t)
            v = kq_proj(t)
        if c < 3:
            g_acc(c)
    anchor(1, v)

    wait(g_u)
    w_transpose(wvT, 0, 2)
    for m in range(D // 128):
        _stb(woT, m * 128, 0, wo_v[:, m * 128:(m + 1) * 128].T)
    g_acc(3)
    z_done = z_sum()
    kvs = None
    for j in range(F // UN):
        if j in W1_CUTS[1:-1]:
            wait(g_w1 + W1_CUTS.index(j) - 1)
        if j == F // UN - 1:
            anchor(2, v)
            wait(g_y)
        v = u_proj(j, z_done if j == 2 else None)
        if j == 0:
            kvs = kv_blocks()
        if j == 1:
            m_matrix(kvs)

    for t in range(NTILE):
        pq_norm(t, out_done(outs[t - 1]) if t > 0 else None)
        out_tile(t)
    for c in c_o:
        c.wait()


def make():
    @jax.jit
    def fn(A_x, A_wqkv, A_wo, B_x, B_w1, B_b1, B_w2, B_b2, gate_w):
        del B_x
        any_spec = pl.BlockSpec(memory_space=pl.ANY)
        return pl.pallas_call(
            _kernel,
            out_shape=jax.ShapeDtypeStruct((1, S, D), BF),
            in_specs=[any_spec] * 8,
            out_specs=any_spec,
            scratch_shapes=[
                pltpu.VMEM((S, D), BF),
                pltpu.VMEM((D, 3 * D), BF),
                pltpu.VMEM((D, D), BF),
                pltpu.VMEM((S, F), BF),
                pltpu.VMEM((F, S), BF),
                pltpu.VMEM((F,), BF),
                pltpu.VMEM((S,), BF),
                pltpu.VMEM((D,), BF),
                pltpu.VMEM((D + 8, D), U32),
                pltpu.VMEM((D // 2, D), U32),
                pltpu.VMEM((D // 2, D), U32),
                pltpu.VMEM((D // 2, S), U32),
                pltpu.VMEM((D // 2, S), U32),
                pltpu.VMEM((D // 2, S), U32),
                pltpu.VMEM((D // 2, S), U32),
                pltpu.VMEM((D // 2, F), U32),
                pltpu.VMEM((D // 2, D), U32),
                pltpu.VMEM((8, S), F32),
                pltpu.VMEM((D, D), F32),
                pltpu.VMEM((D, T), F32),
                pltpu.VMEM((8, T), F32),
                pltpu.SemaphoreType.DMA((N_DMA_GROUPS + 1,)),
            ] + [pltpu.VMEM((32, T), BF)] * 3
              + [pltpu.VMEM((T, D), BF)] * NTILE,
            compiler_params=pltpu.CompilerParams(
                vmem_limit_bytes=100 * 1024 * 1024,
                disable_semaphore_checks=True,
                flags={"XLA_TPU_RESCHEDULE_DMA_DONES": True},
            ),
        )(A_x, A_wqkv, A_wo, B_w1, B_b1, B_w2, B_b2, gate_w)

    return fn


_fn = make()


def pallas_gated_mix__linear_attn_block__mixer_token_mlp__prompt_kernel(A_x, A_wqkv, A_wo, B_x, B_w1, B_b1, B_w2, B_b2, gate_w):
    return _fn(A_x, A_wqkv, A_wo, B_x, B_w1, B_b1, B_w2, B_b2, gate_w)
```
